```python
import jax
import jax.numpy as jnp

def _softmax(x, axis=-1):
    return jax.nn.softmax(x, axis=axis)

def _gelu(x):
    return jax.nn.gelu(x, approximate=True)

def _silu(x):
    return jax.nn.silu(x)

def _sigmoid(x):
    return jax.nn.sigmoid(x)

def _layernorm(x, axis=-1, eps=1e-05):
    m = jnp.mean(x, axis=axis, keepdims=True)
    v = jnp.var(x, axis=axis, keepdims=True)
    return (x - m) / jnp.sqrt(v + eps)

def _scatter_add(tgt, idx, src, axis=0):
    return tgt.at[idx].add(src)

def _segment_sum(src, seg, n):
    return jax.ops.segment_sum(src, seg, n)

class _Rng:

    def __init__(self, key):
        self._k = key

    def _next(self):
        self._k, sub = jax.random.split(self._k)
        return sub

    def normal(self, shape):
        return jax.random.normal(self._next(), shape, dtype=jnp.bfloat16)

    def randint(self, lo, hi, shape):
        return jax.random.randint(self._next(), shape, lo, hi, dtype=jnp.int32)

    def uniform(self, shape, lo=0.0, hi=1.0):
        return jax.random.uniform(self._next(), shape, jnp.bfloat16, lo, hi)

    def permutation(self, n):
        return jax.random.permutation(self._next(), n)
kernel_name = 'adaLN_cond__sliding_block_cached__mixer_token_mlp__decode'

def setup_inputs():
    _rng = _Rng(jax.random.key(int.from_bytes(__import__("os").urandom(4), "little")))
    _w = lambda a: (lambda t: t.astype(jnp.bfloat16) if jnp.issubdtype(t.dtype, jnp.floating) else t)(jnp.asarray(a))

    def _A_setup():
        B, Sq, D = (1, 1, 640)
        Hq, Hkv, Sk, Dh = (32, 32, 32768, 192)
        assert Hq % Hkv == 0, (Hq, Hkv)
        return {'x': _w((lambda *s: _rng.normal(s) * 0.05)(B, Sq, D)), 'k_cache': _w((lambda *s: _rng.normal(s) * 0.05)(B, Hkv, Sk, Dh)), 'v_cache': _w((lambda *s: _rng.normal(s) * 0.05)(B, Hkv, Sk, Dh)), 'wq': _w((lambda *s: _rng.normal(s) * 0.05)(D, Hq * Dh) * D ** (-0.5)), 'wo': _w((lambda *s: _rng.normal(s) * 0.05)(Hq * Dh, D) * (Hq * Dh) ** (-0.5))}
    _A_in = _A_setup()

    def _B_setup():
        B, S, D, F = (1, 1, 640, 1536)
        return {'x': _w((lambda *s: _rng.normal(s) * 0.05)(B, S, D)), 'w1': _w((lambda *s: _rng.normal(s) * 0.05)(S, F) * S ** (-0.5)), 'b1': _w((lambda *s: _rng.normal(s) * 0.05)(F) * 0.02), 'w2': _w((lambda *s: _rng.normal(s) * 0.05)(F, S) * F ** (-0.5)), 'b2': _w((lambda *s: _rng.normal(s) * 0.05)(S) * 0.02)}
    _B_in = _B_setup()
    return {'A_x': _A_in['x'], 'A_k_cache': _A_in['k_cache'], 'A_v_cache': _A_in['v_cache'], 'A_wq': _A_in['wq'], 'A_wo': _A_in['wo'], 'B_x': _B_in['x'], 'B_w1': _B_in['w1'], 'B_b1': _B_in['b1'], 'B_w2': _B_in['w2'], 'B_b2': _B_in['b2'], 'c': _w((lambda *s: _rng.normal(s) * 0.05)(1, 640)), 'w_mod': _w((lambda *s: _rng.normal(s) * 0.05)(640, 6 * 640) * 640 ** (-0.5))}

def reference(A_x, A_k_cache, A_v_cache, A_wq, A_wo, B_x, B_w1, B_b1, B_w2, B_b2, c, w_mod):

    def _A_ref(x, k_cache, v_cache, wq, wo):
        B, Sq, D = x.shape
        Hq, Dh = (32, 192)
        Hkv, Sk = (k_cache.shape[1], k_cache.shape[2])
        W = min(4096, max(256, Sk // 4))
        rep = Hq // Hkv
        q = (lambda x, *d: x.transpose(*d))((x @ wq).reshape(B, Sq, Hq, Dh), 0, 2, 1, 3)
        k = jnp.repeat(k_cache[:, :, Sk - W:, :], rep, axis=1)
        v = jnp.repeat(v_cache[:, :, Sk - W:, :], rep, axis=1)
        scores = jnp.einsum('bhqd,bhkd->bhqk', q, k) * Dh ** (-0.5)
        p = _softmax(scores, axis=-1)
        o = jnp.einsum('bhqk,bhkd->bhqd', p, v)
        return (lambda x, *d: x.transpose(*d))(o, 0, 2, 1, 3).reshape(B, Sq, Hq * Dh) @ wo

    def _B_ref(x, w1, b1, w2, b2):
        B, S, D = x.shape
        h = _layernorm(x, axis=-1)
        u = jnp.einsum('bsd,sf->bdf', h, w1) + b1
        u = _gelu(u)
        y = jnp.einsum('bdf,fs->bds', u, w2) + b2
        return (lambda x, *d: x.transpose(*d))(y, 0, 2, 1)
    x = A_x
    mod = (_silu(c) @ w_mod).reshape(c.shape[0], 6, 1, -1)
    sa, ca, ga, sb, cb, gb = (mod[:, 0].copy(), mod[:, 1].copy(), mod[:, 2].copy(), mod[:, 3].copy(), mod[:, 4].copy(), mod[:, 5].copy())
    h = _layernorm(x, axis=-1) * (1 + ca) + sa
    x = x + ga * _A_ref(h, A_k_cache, A_v_cache, A_wq, A_wo)
    h = _layernorm(x, axis=-1) * (1 + cb) + sb
    x = x + gb * _B_ref(h, B_w1, B_b1, B_w2, B_b2)
    return x
```

```python
import jax
import jax.numpy as jnp
from jax import lax
import jax.experimental.pallas as pl
import jax.experimental.pallas.tpu as pltpu

_EPS = 1e-05
_DEPTH = 6


def _layernorm(x):
    m = jnp.mean(x, axis=-1, keepdims=True)
    d = x - m
    v = jnp.mean(d * d, axis=-1, keepdims=True)
    return d / jnp.sqrt(v + _EPS)


def _col_bcast(row):
    return jnp.broadcast_to(row, (128, row.shape[1])).T


@jax.jit
def pallas_adaLN_cond__sliding_block_cached__mixer_token_mlp__decode_kernel(
    A_x: jax.Array,
    A_k_cache: jax.Array,
    A_v_cache: jax.Array,
    A_wq: jax.Array,
    A_wo: jax.Array,
    B_x: jax.Array,
    B_w1: jax.Array,
    B_b1: jax.Array,
    B_w2: jax.Array,
    B_b2: jax.Array,
    c: jax.Array,
    w_mod: jax.Array,
):
    del B_x
    _, _, D = A_x.shape
    _, H, Sk, Dh = A_k_cache.shape
    F = B_w1.shape[1]
    W = min(4096, max(256, Sk // 4))
    scale = Dh ** (-0.5)
    depth = _DEPTH
    bf16, f32 = jnp.bfloat16, jnp.float32

    def body(x_hbm, kt_hbm, vt_hbm, wq_hbm, wo_hbm, w1_hbm, b1_hbm, w2_hbm, b2_hbm,
             c_hbm, wm_hbm, o_ref,
             x_v, c_v, w1_v, b1_v, w2_v, b2_v, wm_v, wq_v, wo_v, kb, vb,
             q_s, w1c, b1c, w2c, s_small, s_w, s_k, s_v, s_wo):

        def k_cp(h, slot):
            return pltpu.make_async_copy(
                kt_hbm.at[h, :, pl.ds(Sk - W, W)], kb.at[slot], s_k.at[slot])

        def v_cp(h, slot):
            return pltpu.make_async_copy(
                vt_hbm.at[h, :, pl.ds(Sk - W, W)], vb.at[slot], s_v.at[slot])

        def wo_cp(h):
            r = pl.ds(pl.multiple_of(h * Dh, Dh), Dh)
            return pltpu.make_async_copy(wo_hbm.at[r], wo_v.at[r], s_wo.at[h])

        small = [
            pltpu.make_async_copy(src, dst, s_small.at[i])
            for i, (src, dst) in enumerate((
                (c_hbm, c_v), (x_hbm, x_v), (w1_hbm, w1_v), (b1_hbm, b1_v),
                (w2_hbm, w2_v), (b2_hbm, b2_v)))
        ]
        wm_a = pltpu.make_async_copy(
            wm_hbm.at[:, pl.ds(0, 2 * D)], wm_v.at[:, pl.ds(0, 2 * D)], s_w.at[0])
        wm_b = pltpu.make_async_copy(
            wm_hbm.at[:, pl.ds(2 * D, 4 * D)], wm_v.at[:, pl.ds(2 * D, 4 * D)], s_w.at[1])
        wq_cp = pltpu.make_async_copy(wq_hbm, wq_v, s_w.at[2])

        wm_a.start()
        for cp in small:
            cp.start()
        wq_cp.start()
        wm_b.start()
        for h in range(depth):
            k_cp(h, h).start()
            v_cp(h, h).start()
            wo_cp(h).start()

        small[0].wait()
        cv = c_v[...].astype(f32)
        sc = jnp.broadcast_to(cv * jax.nn.sigmoid(cv), (16, D)).astype(bf16)
        wm_a.wait()
        mod_a = jnp.dot(sc, wm_v[:, 0:2 * D], preferred_element_type=f32)[0:1]
        sa, ca = mod_a[:, 0:D], mod_a[:, D:2 * D]
        small[1].wait()
        x = x_v[...].astype(f32)
        h1 = _layernorm(x) * (1.0 + ca) + sa
        wq_cp.wait()
        q = jnp.dot(jnp.broadcast_to(h1, (16, D)).astype(bf16), wq_v[...],
                    preferred_element_type=f32)
        for h in range(H):
            q_s[h] = q[:, h * Dh:(h + 1) * Dh].astype(bf16)

        wm_b.wait()
        mod_b = jnp.dot(sc, wm_v[:, 2 * D:6 * D], preferred_element_type=f32)[0:1]
        ga, sb, cb, gb = (mod_b[:, i * D:(i + 1) * D] for i in range(4))
        for cp in small[2:]:
            cp.wait()
        w1c[...] = _col_bcast(w1_v[...].astype(f32))
        b1c[...] = _col_bcast(b1_v[...].astype(f32).reshape(1, F))
        w2c[...] = _col_bcast(w2_v[...].astype(f32))

        def head(h, acc):
            slot = lax.rem(h, depth)
            k_cp(h, slot).wait()
            s = jnp.dot(q_s[h], kb[slot], preferred_element_type=f32) * scale

            @pl.when(h + depth < H)
            def _():
                k_cp(h + depth, slot).start()

            m = jnp.max(s, axis=-1, keepdims=True)
            p = jnp.exp(s - m)
            l = jnp.sum(p, axis=-1, keepdims=True)
            v_cp(h, slot).wait()
            o = lax.dot_general(p.astype(bf16), vb[slot], (((1,), (1,)), ((), ())),
                                preferred_element_type=f32)

            @pl.when(h + depth < H)
            def _():
                v_cp(h + depth, slot).start()
                wo_cp(h + depth).start()

            o = (o / l).astype(bf16)
            wo_cp(h).wait()
            r = pl.ds(pl.multiple_of(h * Dh, Dh), Dh)
            return acc + jnp.dot(o, wo_v[r], preferred_element_type=f32)

        attn = lax.fori_loop(0, H, head, jnp.zeros((16, D), f32))[0:1]

        x1 = x + ga * attn
        h2 = _layernorm(x1) * (1.0 + cb) + sb
        h3 = _layernorm(h2)
        hb = jnp.broadcast_to(h3, (8, D))

        c1 = 0.7978845608028654
        c2 = c1 * 0.044715
        rows = 64

        def mlp(i, acc):
            r = pl.ds(pl.multiple_of(i * rows, rows), rows)
            w1b, b1b, w2b = w1c[r], b1c[r], w2c[r]
            outs = []
            for j in range(D // 128):
                hj = jnp.broadcast_to(h3[:, j * 128:(j + 1) * 128], (rows, 128))
                u = hj * w1b + b1b
                t = jnp.tanh(u * (c1 + c2 * (u * u)))
                g = (u * w2b) * (1.0 + t)
                outs.append(acc[j] + g.reshape(rows // 8, 8, 128).sum(axis=0))
            return tuple(outs)

        accs = lax.fori_loop(0, F // rows, mlp,
                             tuple(jnp.zeros((8, 128), f32) for _ in range(D // 128)))
        y = jnp.concatenate([a.sum(axis=0, keepdims=True) for a in accs], axis=1)
        y = 0.5 * y + b2_v[...].astype(f32)
        o_ref[...] = (x1 + gb * y).astype(o_ref.dtype)

    any_spec = pl.BlockSpec(memory_space=pl.ANY)
    out = pl.pallas_call(
        body,
        out_shape=jax.ShapeDtypeStruct((1, D), A_x.dtype),
        in_specs=[any_spec] * 11,
        out_specs=pl.BlockSpec(memory_space=pltpu.VMEM),
        scratch_shapes=[
            pltpu.VMEM((1, D), bf16), pltpu.VMEM((1, D), bf16),
            pltpu.VMEM((1, F), bf16), pltpu.VMEM((F,), bf16), pltpu.VMEM((1, F), bf16),
            pltpu.VMEM((1, 1), bf16),
            pltpu.VMEM((D, 6 * D), bf16), pltpu.VMEM((D, H * Dh), bf16),
            pltpu.VMEM((H * Dh, D), bf16),
            pltpu.VMEM((depth, Dh, W), bf16), pltpu.VMEM((depth, Dh, W), bf16),
            pltpu.VMEM((H, 16, Dh), bf16),
            pltpu.VMEM((F, 128), f32), pltpu.VMEM((F, 128), f32), pltpu.VMEM((F, 128), f32),
            pltpu.SemaphoreType.DMA((6,)), pltpu.SemaphoreType.DMA((3,)),
            pltpu.SemaphoreType.DMA((depth,)), pltpu.SemaphoreType.DMA((depth,)),
            pltpu.SemaphoreType.DMA((H,)),
        ],
        compiler_params=pltpu.CompilerParams(vmem_limit_bytes=100 * 1024 * 1024),
    )(
        A_x.reshape(1, D),
        jnp.swapaxes(A_k_cache, 2, 3).reshape(H, Dh, Sk),
        jnp.swapaxes(A_v_cache, 2, 3).reshape(H, Dh, Sk),
        A_wq, A_wo, B_w1, B_b1, B_w2.reshape(1, F), B_b2.reshape(1, 1), c, w_mod,
    )
    return out.reshape(A_x.shape)
```

```python
import jax
import jax.numpy as jnp
from jax import lax
import jax.experimental.pallas as pl
import jax.experimental.pallas.tpu as pltpu

_EPS = 1e-05
_DEPTH = 3
_MLP_ROWS = 256
_KV_ROWS, _KV_COLS = 32, 512


def _layernorm(x):
    m = jnp.mean(x, axis=-1, keepdims=True)
    d = x - m
    v = jnp.mean(d * d, axis=-1, keepdims=True)
    return d / jnp.sqrt(v + _EPS)


def _col_bcast(row):
    return jnp.broadcast_to(row, (128, row.shape[1])).T


@jax.jit
def pallas_adaLN_cond__sliding_block_cached__mixer_token_mlp__decode_kernel(
    A_x: jax.Array,
    A_k_cache: jax.Array,
    A_v_cache: jax.Array,
    A_wq: jax.Array,
    A_wo: jax.Array,
    B_x: jax.Array,
    B_w1: jax.Array,
    B_b1: jax.Array,
    B_w2: jax.Array,
    B_b2: jax.Array,
    c: jax.Array,
    w_mod: jax.Array,
):
    del B_x
    _, _, D = A_x.shape
    _, H, Sk, Dh = A_k_cache.shape
    F = B_w1.shape[1]
    W = min(4096, max(256, Sk // 4))
    scale = Dh ** (-0.5)
    depth = _DEPTH
    bf16, f32 = jnp.bfloat16, jnp.float32

    def body(x_hbm, kt_hbm, vt_hbm, wq_hbm, wo_hbm, w1_hbm, b1_hbm, w2_hbm, b2_hbm,
             c_hbm, wm_hbm, o_ref,
             x_v, c_v, w1_v, b1_v, w2_v, b2_v, wm_v, wq_v, wo_v, kb, vb,
             q_s, w1c, b1c, w2c, s_w, s_k, s_v, s_wo):

        def kv_start(h, slot):
            def col(j, carry):
                cols = pl.multiple_of(j * _KV_COLS, _KV_COLS)
                for i in range(Dh // _KV_ROWS):
                    rows = pl.ds(i * _KV_ROWS, _KV_ROWS)
                    for prio, (src, buf, sem) in enumerate(((kt_hbm, kb, s_k), (vt_hbm, vb, s_v))):
                        pltpu.make_async_copy(
                            src.at[h, rows, pl.ds(Sk - W + cols, _KV_COLS)],
                            buf.at[slot, rows, pl.ds(cols, _KV_COLS)],
                            sem.at[slot]).start(priority=prio)
                return carry
            lax.fori_loop(0, W // _KV_COLS, col, 0)

        def kv_wait(buf, sem, slot):
            pltpu.make_async_copy(buf.at[slot], buf.at[slot], sem.at[slot]).wait()

        def w_start(src, dst, sem, row0, nrows, col0, ncols, pr, pc):
            def piece(i, carry):
                for prio in range(2):
                    rows = pl.ds(pl.multiple_of(row0 + prio * (nrows // 2) + i * pr, pr), pr)
                    for j in range(ncols // pc):
                        cols = pl.ds(col0 + j * pc, pc)
                        pltpu.make_async_copy(
                            src.at[rows, cols], dst.at[rows, cols], sem).start(priority=prio)
                return carry
            lax.fori_loop(0, nrows // 2 // pr, piece, 0)

        def wo_rows(h):
            return pl.ds(pl.multiple_of(h * Dh, Dh), Dh)

        def wo_start(h, slot):
            w_start(wo_hbm, wo_v, s_wo.at[slot], h * Dh, Dh, 0, D, 32, D)

        def wo_wait(h, slot):
            blk = wo_v.at[wo_rows(h)]
            pltpu.make_async_copy(blk, blk, s_wo.at[slot]).wait()

        def wm_start(lo, n, i):
            w_start(wm_hbm, wm_v, s_w.at[i], 0, D, lo * D, n * D, 32, D)

        def wm_wait(lo, n, i):
            blk = wm_v.at[:, pl.ds(lo * D, n * D)]
            pltpu.make_async_copy(blk, blk, s_w.at[i]).wait()

        small = [
            pltpu.make_async_copy(src, dst, s_w.at[4])
            for src, dst in ((c_hbm, c_v), (x_hbm, x_v), (w1_hbm, w1_v), (b1_hbm, b1_v),
                             (w2_hbm, w2_v), (b2_hbm, b2_v))
        ]

        wm_start(0, 2, 0)
        for cp in small:
            cp.start()
        w_start(wq_hbm, wq_v, s_w.at[3], 0, D, 0, H * Dh, 16, 1024)
        kv_start(0, 0)

        for cp in small:
            cp.wait()
        cv = c_v[...].astype(f32)
        sc = jnp.broadcast_to(cv * jax.nn.sigmoid(cv), (16, D)).astype(bf16)
        wm_wait(0, 2, 0)
        mod_a = jnp.dot(sc, wm_v[:, 0:2 * D], preferred_element_type=f32)[0:8]
        sa, ca = mod_a[:, 0:D], mod_a[:, D:2 * D]
        x = jnp.broadcast_to(x_v[...].astype(f32), (8, D))
        h1 = _layernorm(x) * (1.0 + ca) + sa
        pltpu.make_async_copy(wq_v, wq_v, s_w.at[3]).wait()
        q = jnp.dot(jnp.concatenate([h1, h1], axis=0).astype(bf16), wq_v[...],
                    preferred_element_type=f32)
        for h in range(H):
            q_s[h] = q[:, h * Dh:(h + 1) * Dh].astype(bf16)

        wm_start(2, 3, 1)
        for h in range(1, depth):
            kv_start(h, h)
            wo_start(h - 1, h - 1)
        wm_wait(2, 3, 1)
        mod_b = jnp.dot(sc, wm_v[:, 2 * D:5 * D], preferred_element_type=f32)[0:8]
        ga, sb, cb = (mod_b[:, i * D:(i + 1) * D] for i in range(3))

        c1 = 0.7978845608028654
        r = (c1 * 0.044715) ** (1.0 / 3.0)
        kappa = c1 / r
        w1s = w1_v[...].astype(f32) * r
        b1s = b1_v[...].astype(f32).reshape(1, F) * r
        w2s = w2_v[...].astype(f32) * (0.5 / r)
        w1c[...] = _col_bcast(w1s)
        b1c[...] = _col_bcast(b1s)
        w2c[...] = _col_bcast(w2s)
        lin_w = jnp.sum(w1s * w2s, axis=-1, keepdims=True)
        lin_b = jnp.sum(b1s * w2s, axis=-1, keepdims=True) + b2_v[...].astype(f32)

        def out_proj(h, o):
            wo_wait(h, lax.rem(h, depth))
            return jnp.dot(o, wo_v[wo_rows(h)], preferred_element_type=f32)[0:8]

        def head(h, carry):
            acc, o_prev = carry
            slot = lax.rem(h, depth)
            kv_wait(kb, s_k, slot)
            s = jnp.dot(q_s[h], kb[slot], preferred_element_type=f32) * scale

            m = jnp.max(s, axis=-1, keepdims=True)
            p = jnp.exp(s - m)
            l = jnp.sum(p, axis=-1, keepdims=True)
            kv_wait(vb, s_v, slot)
            o = lax.dot_general(p.astype(bf16), vb[slot], (((1,), (1,)), ((), ())),
                                preferred_element_type=f32)
            o = (o / l).astype(bf16)

            acc = lax.cond(h > 0, lambda: acc + out_proj(h - 1, o_prev), lambda: acc)

            @pl.when(h + depth < H)
            def _():
                kv_start(h + depth, slot)
                wo_start(h + depth - 1, lax.rem(h + depth - 1, depth))

            @pl.when(h == H - depth + 1)
            def _():
                wo_start(H - 1, (H - 1) % depth)
                wm_start(5, 1, 2)

            return acc, o

        acc, o_last = lax.fori_loop(
            0, H, head, (jnp.zeros((8, D), f32), jnp.zeros((16, Dh), bf16)))
        attn = acc + out_proj(H - 1, o_last)

        x1 = x + ga * attn
        h2 = _layernorm(x1) * (1.0 + cb) + sb
        h3 = _layernorm(h2)
        rows = _MLP_ROWS
        hs = [jnp.concatenate([h3[:, j * 128:(j + 1) * 128]] * (rows // 8), axis=0)
              for j in range(D // 128)]

        def mlp(i, acc):
            rr = pl.ds(pl.multiple_of(i * rows, rows), rows)
            w1b, b1b, w2b = w1c[rr], b1c[rr], w2c[rr]
            outs = []
            for j in range(D // 128):
                v = hs[j] * w1b + b1b
                g = (v * w2b) * jnp.tanh(v * (v * v + kappa))
                a = acc[j]
                for k in range(rows // 8):
                    a = a + g[k * 8:(k + 1) * 8]
                outs.append(a)
            return tuple(outs)

        accs = lax.fori_loop(0, F // rows, mlp,
                             tuple(jnp.zeros((8, 128), f32) for _ in range(D // 128)))
        y = jnp.concatenate(accs, axis=1).sum(axis=0, keepdims=True)
        y = y + (h3[0:1] * lin_w + lin_b)
        wm_wait(5, 1, 2)
        gb = jnp.dot(sc, wm_v[:, 5 * D:6 * D], preferred_element_type=f32)[0:1]
        o_ref[...] = (x1[0:1] + gb * y).astype(o_ref.dtype)

    any_spec = pl.BlockSpec(memory_space=pl.ANY)
    out = pl.pallas_call(
        body,
        out_shape=jax.ShapeDtypeStruct((1, D), A_x.dtype),
        in_specs=[any_spec] * 11,
        out_specs=pl.BlockSpec(memory_space=pltpu.VMEM),
        scratch_shapes=[
            pltpu.VMEM((1, D), bf16), pltpu.VMEM((1, D), bf16),
            pltpu.VMEM((1, F), bf16), pltpu.VMEM((F,), bf16), pltpu.VMEM((1, F), bf16),
            pltpu.VMEM((1, 1), bf16),
            pltpu.VMEM((D, 6 * D), bf16), pltpu.VMEM((D, H * Dh), bf16),
            pltpu.VMEM((H * Dh, D), bf16),
            pltpu.VMEM((depth, Dh, W), bf16), pltpu.VMEM((depth, Dh, W), bf16),
            pltpu.VMEM((H, 16, Dh), bf16),
            pltpu.VMEM((F, 128), f32), pltpu.VMEM((F, 128), f32), pltpu.VMEM((F, 128), f32),
            pltpu.SemaphoreType.DMA((5,)),
            pltpu.SemaphoreType.DMA((depth,)), pltpu.SemaphoreType.DMA((depth,)),
            pltpu.SemaphoreType.DMA((depth,)),
        ],
        compiler_params=pltpu.CompilerParams(vmem_limit_bytes=100 * 1024 * 1024),
    )(
        A_x.reshape(1, D),
        jnp.swapaxes(A_k_cache, 2, 3).reshape(H, Dh, Sk),
        jnp.swapaxes(A_v_cache, 2, 3).reshape(H, Dh, Sk),
        A_wq, A_wo, B_w1, B_b1, B_w2.reshape(1, F), B_b2.reshape(1, 1), c, w_mod,
    )
    return out.reshape(A_x.shape)
```

```python
import jax
import jax.numpy as jnp
from jax import lax
import jax.experimental.pallas as pl
import jax.experimental.pallas.tpu as pltpu

_EPS = 1e-05
_DEPTH = 3
_MLP_ROWS = 256
_KV_ROWS, _KV_COLS = 32, 512


def _layernorm(x):
    m = jnp.mean(x, axis=-1, keepdims=True)
    d = x - m
    v = jnp.mean(d * d, axis=-1, keepdims=True)
    return d / jnp.sqrt(v + _EPS)


def _col_bcast(row):
    return jnp.broadcast_to(row, (128, row.shape[1])).T


@jax.jit
def pallas_adaLN_cond__sliding_block_cached__mixer_token_mlp__decode_kernel(
    A_x: jax.Array,
    A_k_cache: jax.Array,
    A_v_cache: jax.Array,
    A_wq: jax.Array,
    A_wo: jax.Array,
    B_x: jax.Array,
    B_w1: jax.Array,
    B_b1: jax.Array,
    B_w2: jax.Array,
    B_b2: jax.Array,
    c: jax.Array,
    w_mod: jax.Array,
):
    del B_x
    _, _, D = A_x.shape
    _, H, Sk, Dh = A_k_cache.shape
    F = B_w1.shape[1]
    W = min(4096, max(256, Sk // 4))
    scale = Dh ** (-0.5)
    depth = _DEPTH
    bf16, f32 = jnp.bfloat16, jnp.float32

    def body(x_hbm, kt_hbm, vt_hbm, wq_hbm, wo_hbm, w1_hbm, b1_hbm, w2_hbm, b2_hbm,
             c_hbm, wm_hbm, o_ref,
             x_v, c_v, w1_v, b1_v, w2_v, b2_v, wm_v, wq_v, wo_v, kb, vb,
             q_s, sc_s, mod_s, w1c, b1c, w2c, s_w, s_k, s_v, s_wo):

        def kv_start(h, slot, j0=0, j1=W // _KV_COLS):
            def col(j, carry):
                cols = pl.multiple_of(j * _KV_COLS, _KV_COLS)
                for i in range(Dh // _KV_ROWS):
                    rows = pl.ds(i * _KV_ROWS, _KV_ROWS)
                    for prio, (src, buf, sem) in enumerate(((kt_hbm, kb, s_k), (vt_hbm, vb, s_v))):
                        pltpu.make_async_copy(
                            src.at[h, rows, pl.ds(Sk - W + cols, _KV_COLS)],
                            buf.at[slot, rows, pl.ds(cols, _KV_COLS)],
                            sem.at[slot]).start(priority=prio)
                return carry
            lax.fori_loop(j0, j1, col, 0)

        def kv_wait(buf, sem, slot):
            pltpu.make_async_copy(buf.at[slot], buf.at[slot], sem.at[slot]).wait()

        def w_start(src, dst, sem, row0, nrows, col0, ncols, pr, pc, prios=(0, 1)):
            def piece(i, carry):
                for prio in range(2):
                    rows = pl.ds(pl.multiple_of(row0 + prio * (nrows // 2) + i * pr, pr), pr)
                    for j in range(ncols // pc):
                        cols = pl.ds(col0 + j * pc, pc)
                        pltpu.make_async_copy(
                            src.at[rows, cols], dst.at[rows, cols], sem).start(priority=prios[prio])
                return carry
            lax.fori_loop(0, nrows // 2 // pr, piece, 0)

        def wo_rows(h):
            return pl.ds(pl.multiple_of(h * Dh, Dh), Dh)

        def wo_start(h, slot, prios=(0, 1)):
            w_start(wo_hbm, wo_v, s_wo.at[slot], h * Dh, Dh, 0, D, 32, D, prios)

        def wo_wait(h, slot):
            blk = wo_v.at[wo_rows(h)]
            pltpu.make_async_copy(blk, blk, s_wo.at[slot]).wait()

        def wm_start(lo, n, i, prios=(0, 1)):
            w_start(wm_hbm, wm_v, s_w.at[i], 0, D, lo * D, n * D, 32, D, prios)

        def wm_wait(lo, n, i):
            blk = wm_v.at[:, pl.ds(lo * D, n * D)]
            pltpu.make_async_copy(blk, blk, s_w.at[i]).wait()

        small = [
            pltpu.make_async_copy(src, dst, s_w.at[4])
            for src, dst in ((c_hbm, c_v), (x_hbm, x_v), (w1_hbm, w1_v), (b1_hbm, b1_v),
                             (w2_hbm, w2_v), (b2_hbm, b2_v))
        ]

        wm_start(0, 2, 0)
        for cp in small:
            cp.start()
        w_start(wq_hbm, wq_v, s_w.at[3], 0, D, 0, 2048, 16, 1024)
        for cp in small:
            cp.wait()
        cv = c_v[...].astype(f32)
        sc = jnp.broadcast_to(cv * jax.nn.sigmoid(cv), (16, D)).astype(bf16)
        sc_s[...] = sc
        wm_wait(0, 2, 0)
        mod_a = jnp.dot(sc, wm_v[:, 0:2 * D], preferred_element_type=f32)[0:8]
        sa, ca = mod_a[:, 0:D], mod_a[:, D:2 * D]
        x = jnp.broadcast_to(x_v[...].astype(f32), (8, D))
        h1 = _layernorm(x) * (1.0 + ca) + sa
        h1 = jnp.concatenate([h1, h1], axis=0).astype(bf16)
        w_start(wq_hbm, wq_v, s_w.at[3], 0, D, 2048, H * Dh - 2048, 16, 1024)
        kv_start(0, 0)
        pltpu.make_async_copy(wq_v, wq_v, s_w.at[3]).wait()
        nq = 8
        nj = W // _KV_COLS
        for i in range(nq):
            hq = H // nq
            q = jnp.dot(h1, wq_v[:, i * hq * Dh:(i + 1) * hq * Dh], preferred_element_type=f32)
            for h in range(hq):
                q_s[i * hq + h] = q[:, h * Dh:(h + 1) * Dh].astype(bf16)
            kv_start(1, 1, i * nj // nq, (i + 1) * nj // nq)
        wm_start(2, 3, 1)
        wo_start(0, 0)

        c1 = 0.7978845608028654
        r = (c1 * 0.044715) ** (1.0 / 3.0)
        kappa = c1 / r
        w1s = lambda: w1_v[...].astype(f32) * r
        b1s = lambda: b1_v[...].astype(f32).reshape(1, F) * r
        w2s = lambda: w2_v[...].astype(f32) * (0.5 / r)

        def side_work(h):
            @pl.when(h == 1)
            def _():
                wm_wait(2, 3, 1)
            for i in range(3):
                @pl.when(h == 1 + i)
                def _():
                    mod_s[:, i * D:(i + 1) * D] = jnp.dot(
                        sc_s[...], wm_v[:, (2 + i) * D:(3 + i) * D],
                        preferred_element_type=f32)[0:8]
            for i, (dst, row) in enumerate(((w1c, w1s), (b1c, b1s), (w2c, w2s))):
                @pl.when(h == 4 + i)
                def _():
                    dst[...] = _col_bcast(row())

        def out_proj(h, o):
            wo_wait(h, lax.rem(h, depth))
            return jnp.dot(o, wo_v[wo_rows(h)], preferred_element_type=f32)[0:8]

        def head(h, carry):
            acc, o_prev = carry
            slot = lax.rem(h, depth)
            kv_wait(kb, s_k, slot)
            s = jnp.dot(q_s[h], kb[slot], preferred_element_type=f32) * scale

            nslot = lax.rem(h + 2, depth)

            @pl.when(h + 2 < H)
            def _():
                kv_start(h + 2, nslot, 0, nj // 2)

            m = jnp.max(s, axis=-1, keepdims=True)
            p = jnp.exp(s - m)
            l = jnp.sum(p, axis=-1, keepdims=True)
            kv_wait(vb, s_v, slot)
            o = lax.dot_general(p.astype(bf16), vb[slot], (((1,), (1,)), ((), ())),
                                preferred_element_type=f32)
            o = (o / l).astype(bf16)

            acc = lax.cond(h > 0, lambda: acc + out_proj(h - 1, o_prev), lambda: acc)

            @pl.when(h + 2 < H)
            def _():
                kv_start(h + 2, nslot, nj // 2, nj)

            @pl.when(h + 1 < H)
            def _():
                wo_start(h + 1, lax.rem(h + 1, depth), (1, 1))

            @pl.when(h == H - 2)
            def _():
                wm_start(5, 1, 2, (1, 1))

            side_work(h)
            return acc, o

        acc, o_last = lax.fori_loop(
            0, H, head, (jnp.zeros((8, D), f32), jnp.zeros((16, Dh), bf16)))
        attn = acc + out_proj(H - 1, o_last)

        ga, sb, cb = (mod_s[:, i * D:(i + 1) * D] for i in range(3))
        lin_w = jnp.sum(w1s() * w2s(), axis=-1, keepdims=True)
        lin_b = jnp.sum(b1s() * w2s(), axis=-1, keepdims=True) + b2_v[...].astype(f32)
        x1 = x + ga * attn
        h2 = _layernorm(x1) * (1.0 + cb) + sb
        h3 = _layernorm(h2)
        rows = _MLP_ROWS
        hs = [jnp.concatenate([h3[:, j * 128:(j + 1) * 128]] * (rows // 8), axis=0)
              for j in range(D // 128)]

        def mlp(i, acc):
            rr = pl.ds(i * rows if isinstance(i, int) else pl.multiple_of(i * rows, rows), rows)
            w1b, b1b, w2b = w1c[rr], b1c[rr], w2c[rr]
            outs = []
            for j in range(D // 128):
                v = hs[j] * w1b + b1b
                g = (v * w2b) * jnp.tanh(v * (v * v + kappa))
                a = acc[j]
                for k in range(rows // 8):
                    a = a + g[k * 8:(k + 1) * 8]
                outs.append(a)
            return tuple(outs)

        n_mlp, n_last = F // rows, 2
        accs = lax.fori_loop(0, n_mlp - n_last, mlp,
                             tuple(jnp.zeros((8, 128), f32) for _ in range(D // 128)))
        wm_wait(5, 1, 2)
        gb = jnp.dot(sc_s[...], wm_v[:, 5 * D:6 * D], preferred_element_type=f32)[0:1]
        for i in range(n_mlp - n_last, n_mlp):
            accs = mlp(i, accs)
        y = jnp.concatenate(accs, axis=1).sum(axis=0, keepdims=True)
        y = y + (h3[0:1] * lin_w + lin_b)
        o_ref[...] = (x1[0:1] + gb * y).astype(o_ref.dtype)

    any_spec = pl.BlockSpec(memory_space=pl.ANY)
    out = pl.pallas_call(
        body,
        out_shape=jax.ShapeDtypeStruct((1, D), A_x.dtype),
        in_specs=[any_spec] * 11,
        out_specs=pl.BlockSpec(memory_space=pltpu.VMEM),
        scratch_shapes=[
            pltpu.VMEM((1, D), bf16), pltpu.VMEM((1, D), bf16),
            pltpu.VMEM((1, F), bf16), pltpu.VMEM((F,), bf16), pltpu.VMEM((1, F), bf16),
            pltpu.VMEM((1, 1), bf16),
            pltpu.VMEM((D, 6 * D), bf16), pltpu.VMEM((D, H * Dh), bf16),
            pltpu.VMEM((H * Dh, D), bf16),
            pltpu.VMEM((depth, Dh, W), bf16), pltpu.VMEM((depth, Dh, W), bf16),
            pltpu.VMEM((H, 16, Dh), bf16), pltpu.VMEM((16, D), bf16), pltpu.VMEM((8, 3 * D), f32),
            pltpu.VMEM((F, 128), f32), pltpu.VMEM((F, 128), f32), pltpu.VMEM((F, 128), f32),
            pltpu.SemaphoreType.DMA((5,)),
            pltpu.SemaphoreType.DMA((depth,)), pltpu.SemaphoreType.DMA((depth,)),
            pltpu.SemaphoreType.DMA((depth,)),
        ],
        compiler_params=pltpu.CompilerParams(vmem_limit_bytes=100 * 1024 * 1024),
    )(
        A_x.reshape(1, D),
        jnp.swapaxes(A_k_cache, 2, 3).reshape(H, Dh, Sk),
        jnp.swapaxes(A_v_cache, 2, 3).reshape(H, Dh, Sk),
        A_wq, A_wo, B_w1, B_b1, B_w2.reshape(1, F), B_b2.reshape(1, 1), c, w_mod,
    )
    return out.reshape(A_x.shape)
```
